```python
import os as _os
_os.environ.setdefault("JAX_PLATFORMS", "cpu")
import jax
import jax.numpy as jnp

def _softmax(x, axis=-1):
    return jax.nn.softmax(x, axis=axis)
def _gelu(x):
    return jax.nn.gelu(x, approximate=True)
def _silu(x):
    return jax.nn.silu(x)
def _sigmoid(x):
    return jax.nn.sigmoid(x)
def _layernorm(x, axis=-1, eps=1e-5):
    m = jnp.mean(x, axis=axis, keepdims=True)
    v = jnp.var(x, axis=axis, keepdims=True)
    return (x - m) / jnp.sqrt(v + eps)
def _scatter_add(tgt, idx, src, axis=0):
    return tgt.at[idx].add(src)
def _segment_sum(src, seg, n):
    return jax.ops.segment_sum(src, seg, n)
class _Rng:
    def __init__(self, key):
        self._k = key
    def _next(self):
        self._k, sub = jax.random.split(self._k)
        return sub
    def normal(self, shape):
        return jax.random.normal(self._next(), shape, dtype=jnp.bfloat16)
    def randint(self, lo, hi, shape):
        return jax.random.randint(self._next(), shape, lo, hi, dtype=jnp.int32)
    def uniform(self, shape, lo=0.0, hi=1.0):
        return jax.random.uniform(self._next(), shape, jnp.bfloat16, lo, hi)
    def permutation(self, n):
        return jax.random.permutation(self._next(), n)


kernel_name = 'concat_heads__mha_block_cached__mha_block_cached__near_ridge'

def setup_inputs():
    _rng = _Rng(jax.random.key(int.from_bytes(__import__("os").urandom(4), "little")))
    _w = (lambda a: (lambda t: t.astype(jnp.bfloat16) if jnp.issubdtype(t.dtype, jnp.floating) else t)(jnp.asarray(a)))
    def _A_setup():
        B, Sq, D = 16, 32, 1024
        H, Sk, Dh = 32, 32, 128
        return {
            "x": _w((lambda *s: _rng.normal(s) * 0.8)(B, Sq, D)),
            "k_cache": _w((lambda *s: _rng.normal(s) * 0.8)(B, H, Sk, Dh)),
            "v_cache": _w((lambda *s: _rng.normal(s) * 0.05)(B, H, Sk, Dh)),
            "wq": _w((lambda *s: _rng.normal(s) * 0.8)(D, H * Dh) * (D ** -0.5)),
            "wo": _w((lambda *s: _rng.normal(s) * 0.05)(H * Dh, D) * ((H * Dh) ** -0.5)),
        }
    _A_in = _A_setup()

    def _B_setup():
        B, Sq, D = 16, 32, 1024
        H, Sk, Dh = 32, 32, 128
        return {
            "x": _w((lambda *s: _rng.normal(s) * 0.8)(B, Sq, D)),
            "k_cache": _w((lambda *s: _rng.normal(s) * 0.8)(B, H, Sk, Dh)),
            "v_cache": _w((lambda *s: _rng.normal(s) * 0.05)(B, H, Sk, Dh)),
            "wq": _w((lambda *s: _rng.normal(s) * 0.8)(D, H * Dh) * (D ** -0.5)),
            "wo": _w((lambda *s: _rng.normal(s) * 0.05)(H * Dh, D) * ((H * Dh) ** -0.5)),
        }
    _B_in = _B_setup()

    return {
        "A_x": _A_in["x"],
        "A_k_cache": _A_in["k_cache"],
        "A_v_cache": _A_in["v_cache"],
        "A_wq": _A_in["wq"],
        "A_wo": _A_in["wo"],
        "B_x": _B_in["x"],
        "B_k_cache": _B_in["k_cache"],
        "B_v_cache": _B_in["v_cache"],
        "B_wq": _B_in["wq"],
        "B_wo": _B_in["wo"],
    }

def reference(A_x, A_k_cache, A_v_cache, A_wq, A_wo, B_x, B_k_cache, B_v_cache, B_wq, B_wo):
    def _A_ref(x, k_cache, v_cache, wq, wo):
        B, Sq, D = x.shape
        H, Dh = 32, 128
        q = (lambda x, *d: x.transpose(*d))((x @ wq).reshape(B, Sq, H, Dh), 0, 2, 1, 3)
        scores = jnp.einsum("bhqd,bhkd->bhqk", q, k_cache) * (Dh ** -0.5)
        p = _softmax(scores, axis=-1)
        o = jnp.einsum("bhqk,bhkd->bhqd", p, v_cache)
        return (lambda x, *d: x.transpose(*d))(o, 0, 2, 1, 3).reshape(B, Sq, H * Dh) @ wo

    def _B_ref(x, k_cache, v_cache, wq, wo):
        B, Sq, D = x.shape
        H, Dh = 32, 128
        q = (lambda x, *d: x.transpose(*d))((x @ wq).reshape(B, Sq, H, Dh), 0, 2, 1, 3)
        scores = jnp.einsum("bhqd,bhkd->bhqk", q, k_cache) * (Dh ** -0.5)
        p = _softmax(scores, axis=-1)
        o = jnp.einsum("bhqk,bhkd->bhqd", p, v_cache)
        return (lambda x, *d: x.transpose(*d))(o, 0, 2, 1, 3).reshape(B, Sq, H * Dh) @ wo

    a = _A_ref(A_x, A_k_cache, A_v_cache, A_wq, A_wo)
    b = _B_ref(B_x, B_k_cache, B_v_cache, B_wq, B_wo)
    return jnp.concatenate([a, b], axis=-1)
```

```python
import jax
import jax.numpy as jnp
from jax import lax
import jax.experimental.pallas as pl
import jax.experimental.pallas.tpu as pltpu

B, SQ, D = 16, 32, 1024
H, SK, DH = 32, 32, 128
M = B * SQ
G = 8
NB = H // G
U = 4
NQ = 4
QW = D // NQ
NX = 2
LOG2E = 1.4426950408889634
SCALE = (DH ** -0.5) * LOG2E

X_BATCHES = [
    [('x', 0, 0), ('wq', 0, 1)],
    [('wq', 1, 3)],
    [('wq', 3, 8)],
    [('wq', 8, 16), ('k', 0, 2), ('v', 0, 2)],
    [('k', 2, 8), ('v', 2, 8), ('wo', 0, 8)],
    [('k', 8, 16), ('v', 8, 16), ('wo', 8, 16)],
]
X_ORDER = (
    "W0 Q0 W1 Q1 Q2 W2 Q3 Q4 Q5 Q6 Q7 "
    "W3 S0 S1 Q8 P0 P1 Q9 Q10 Q11 Q12 Q13 "
    "W4 S2 S3 Q14 P2 P3 S4 S5 Q15 P4 P5 S6 S7 O0.0 P6 P7 O0.1 O0.2 O0.3 O1.0 "
    "W5 S8 S9 O1.1 P8 P9 S10 S11 O1.2 P10 P11 S12 S13 O1.3 P12 P13 S14 S15 O2.0 P14 P15 "
    "O2.1 O2.2 O2.3 O3.0 O3.1 O3.2 O3.3")
LOOP_ORDER = (
    "Q0 Q1 S0 Q2 P0 S1 Q3 P1 S2 Q4 P2 S3 Q5 P3 S4 Q6 P4 S5 Q7 P5 S6 O0.0 P6 S7 O0.1 P7 "
    "O0.2 O0.3 O1.0 O1.1 O1.2 O1.3")
NXD = sum(len(b) for b in X_BATCHES)
NDMA = NXD + 4 * (2 * NB - NX) + 1


def _kernel(ax, ak, av, awq, awo, bx, bk, bv, bwq, bwo, out_hbm,
            x_buf, wq_buf, k_buf, v_buf, wo_buf, q_buf, o_buf, acc, out_buf,
            in_sem, out_sem):
    srcs = ({'x': ax, 'k': ak, 'v': av, 'wq': awq, 'wo': awo},
            {'x': bx, 'k': bk, 'v': bv, 'wq': bwq, 'wo': bwo})

    def in_copy(kind, br, lo, hi, sem_idx):
        src = srcs[br][kind]
        if kind == 'x':
            return pltpu.make_async_copy(src, x_buf.at[br], in_sem.at[sem_idx])
        blk, l0 = br * NB + lo // G, lo % G
        n = hi - lo
        assert l0 + n <= G
        if kind == 'wq':
            s = src.at[:, pl.ds(lo * DH, n * DH)]
            d = wq_buf.at[blk, :, pl.ds(l0 * DH, n * DH)]
        elif kind == 'wo':
            s = src.at[pl.ds(lo * DH, n * DH), :]
            d = wo_buf.at[blk, pl.ds(l0 * DH, n * DH), :]
        else:
            buf = k_buf if kind == 'k' else v_buf
            s = src.at[:, pl.ds(lo, n)]
            d = buf.at[blk, :, pl.ds(l0, n)]
        return pltpu.make_async_copy(s, d, in_sem.at[sem_idx])

    x_copies = []
    n = 0
    for batch in X_BATCHES:
        cps = []
        for kind, lo, hi in batch:
            cp = in_copy(kind, 0, lo, hi, n)
            cp.start()
            cps.append(cp)
            n += 1
        x_copies.append(cps)
    XB_SEM = NDMA - 1
    for blk in range(NX, 2 * NB):
        br, g = divmod(blk, NB)
        if blk == NB:
            in_copy('x', 1, 0, 0, XB_SEM).start()
        for j, kind in enumerate(('wq', 'k', 'v', 'wo')):
            in_copy(kind, br, g * G, (g + 1) * G, NXD + 4 * (blk - NX) + j).start()

    acc[1] = jnp.zeros((M, D), jnp.float32)

    row = lax.broadcasted_iota(jnp.int32, (128, 128), 0) // SQ
    col = lax.broadcasted_iota(jnp.int32, (128, 128), 1) // SK
    mask = row == col

    def run(order, br, blk0, in_loop):
        p = {}

        def qproj(h):
            blk, l = blk0 + h // G, h % G
            qq = jnp.dot(x_buf[br], wq_buf[blk, :, l * DH:(l + 1) * DH],
                         preferred_element_type=jnp.float32)
            q_buf[h] = (qq * SCALE).astype(jnp.bfloat16)

        def scores(h):
            blk, l = blk0 + h // G, h % G
            for j in range(4):
                qs = q_buf[h, j * 128:(j + 1) * 128, :]
                ks = k_buf[blk, pl.ds(4 * j, 4), l].reshape(128, DH)
                sc = lax.dot_general(qs, ks, (((1,), (1,)), ((), ())),
                                     preferred_element_type=jnp.float32)
                sc = jnp.where(mask, sc, -jnp.inf)
                m = jnp.max(sc, axis=-1, keepdims=True)
                e = jnp.exp2(sc - m)
                den = jnp.sum(e, axis=-1, keepdims=True)
                p[h, j] = (e.astype(jnp.bfloat16), pl.reciprocal(den, approx=True))

        def pv(h):
            blk, l = blk0 + h // G, h % G
            for j in range(4):
                vs = v_buf[blk, pl.ds(4 * j, 4), l].reshape(128, DH)
                e, r = p.pop((h, j))
                oo = jnp.dot(e, vs, preferred_element_type=jnp.float32)
                o_buf[h, j * 128:(j + 1) * 128, :] = (oo * r).astype(jnp.bfloat16)

        def oproj(u, c):
            blk, l = blk0 + (u * U) // G, (u * U) % G
            lhs = jnp.concatenate([o_buf[u * U + i] for i in range(U)], axis=1)
            cs = slice(c * QW, (c + 1) * QW)
            y = jnp.dot(lhs, wo_buf[blk, l * DH:(l + U) * DH, cs],
                        preferred_element_type=jnp.float32)
            if not in_loop and u == 0:
                acc[br, :, cs] = y
                return
            y = acc[br, :, cs] + y
            acc[br, :, cs] = y
            if in_loop and u == G // U - 1:
                out_buf[br, :, cs] = y.astype(jnp.bfloat16)

                @pl.when(blk0 % NB == NB - 1)
                def _():
                    off = pl.multiple_of(br * D + c * QW, QW)
                    pltpu.make_async_copy(out_buf.at[br, :, pl.ds(c * QW, QW)],
                                          out_hbm.at[:, pl.ds(off, QW)],
                                          out_sem.at[br * NQ + c]).start()

        for tok in order.split():
            kind, arg = tok[0], tok[1:]
            if kind == 'W':
                for cp in x_copies[int(arg)]:
                    cp.wait()
            elif kind == 'Q':
                qproj(int(arg))
            elif kind == 'S':
                scores(int(arg))
            elif kind == 'P':
                pv(int(arg))
            else:
                u, c = arg.split('.')
                oproj(int(u), int(c))

    run(X_ORDER, 0, 0, False)

    def body(blk, carry):
        br = blk // NB

        @pl.when(blk == NB)
        def _():
            pltpu.make_async_copy(x_buf.at[1], x_buf.at[1], in_sem.at[XB_SEM]).wait()

        base = NXD + 4 * (blk - NX)
        for j, buf in enumerate((wq_buf, k_buf, v_buf, wo_buf)):
            pltpu.make_async_copy(buf.at[blk], buf.at[blk], in_sem.at[base + j]).wait()
        run(LOOP_ORDER, br, blk, True)
        return carry

    lax.fori_loop(NX, 2 * NB, body, 0)

    for br in range(2):
        for c in range(NQ):
            pltpu.make_async_copy(out_buf.at[br, :, pl.ds(c * QW, QW)],
                                  out_hbm.at[:, pl.ds(br * D + c * QW, QW)],
                                  out_sem.at[br * NQ + c]).wait()


@jax.jit
def pallas_concat_heads__mha_block_cached__mha_block_cached__near_ridge_kernel(
    A_x, A_k_cache, A_v_cache, A_wq, A_wo, B_x, B_k_cache, B_v_cache, B_wq, B_wo):
    bf = jnp.bfloat16
    any_spec = pl.BlockSpec(memory_space=pl.ANY)
    out = pl.pallas_call(
        _kernel,
        out_shape=jax.ShapeDtypeStruct((M, 2 * D), bf),
        in_specs=[any_spec] * 10,
        out_specs=any_spec,
        scratch_shapes=[
            pltpu.VMEM((2, M, D), bf),
            pltpu.VMEM((2 * NB, D, G * DH), bf),
            pltpu.VMEM((2 * NB, B, G, SK, DH), bf),
            pltpu.VMEM((2 * NB, B, G, SK, DH), bf),
            pltpu.VMEM((2 * NB, G * DH, D), bf),
            pltpu.VMEM((NX * G, M, DH), bf),
            pltpu.VMEM((NX * G, M, DH), bf),
            pltpu.VMEM((2, M, D), jnp.float32),
            pltpu.VMEM((2, M, D), bf),
            pltpu.SemaphoreType.DMA((NDMA,)),
            pltpu.SemaphoreType.DMA((2 * NQ,)),
        ],
        compiler_params=pltpu.CompilerParams(
            vmem_limit_bytes=100 * 1024 * 1024,
            disable_bounds_checks=True,
            disable_semaphore_checks=True),
    )(A_x.reshape(M, D), A_k_cache, A_v_cache, A_wq, A_wo,
      B_x.reshape(M, D), B_k_cache, B_v_cache, B_wq, B_wo)
    return out.reshape(B, SQ, 2 * D)
```

```python
import jax
import jax.numpy as jnp
from jax import lax
import jax.experimental.pallas as pl
import jax.experimental.pallas.tpu as pltpu

B, SQ, D = 16, 32, 1024
H, SK, DH = 32, 32, 128
M = B * SQ
G = 16
NBODY = 2 * H // G
NE = 6
NL = G - NE
NQB = 5
U = 4
NQ = 4
QW = D // NQ
KT = 128
NK = D // KT
NR = 4
PAD = 128
LOG2E = 1.4426950408889634
SCALE = (DH ** -0.5) * LOG2E

X_SEGS = [
    [('x', 0, 1), ('w', 0, 1, 0, 4)],
    [('w', 0, 1, 4, 12)],
    [('w', 0, 1, 12, 32)],
    [('x', 1, 2), ('w', 1, 2, 0, 32)],
    [('x', 2, 4), ('w', 2, 4, 0, 28)],
    [('w', 2, 4, 28, 32), ('x', 4, 7), ('w', 4, 7, 0, 28)],
    [('w', 4, 7, 28, 32), ('x', 7, 8), ('w', 7, 8, 0, 32), ('xb',), ('wb', 0), ('wb', 1)],
]
LOOP_ORDER = (
    "Q0 S0 S1 Q1 P0 P1 S2 S3 Q2 P2 P3 S4 S5 Q3 P4 P5 Q4 O0.0 "
    "S6 O0.1 P6 S7 O0.2 P7 S8 O0.3 P8 S9 O1.0 P9 S10 O1.1 P10 S11 O1.2 P11 S12 O1.3 P12 "
    "S13 O2.0 P13 S14 O2.1 P14 S15 O2.2 P15 O2.3 O3.0 O3.1 O3.2 O3.3")
NXD = sum(len(b) for b in X_SEGS)
NDMA = NXD + 4 * NBODY
NOUT = NQ - 1 + NR


def _out_pieces():
    pieces = [(0, M, c) for c in range(NQ - 1)]
    pieces += [(r * (M // NR), M // NR, NQ - 1) for r in range(NR)]
    return pieces


def _kernel(ax, ak, av, awq, awo, bx, bk, bv, bwq, bwo, out_hbm,
            x_buf, wqa_buf, wqe_buf, wql_buf, k_buf, v_buf, wo_buf,
            qacc, qe_buf, ql_buf, o_buf, acc, out_buf, in_sem, out_sem):
    i = pl.program_id(0)

    def x_copy(item, sem_idx):
        kind = item[0]
        if kind == 'x':
            cols = pl.ds(item[1] * KT, (item[2] - item[1]) * KT)
            s, d = ax.at[:, cols], x_buf.at[0, :, cols]
        elif kind == 'w':
            rows = pl.ds(item[1] * KT, (item[2] - item[1]) * KT)
            cols = pl.ds(item[3] * DH, (item[4] - item[3]) * DH)
            s, d = awq.at[rows, cols], wqa_buf.at[rows, cols]
        elif kind == 'xb':
            s, d = bx, x_buf.at[1]
        else:
            s = bwq.at[:, pl.ds(item[1] * G * DH, NE * DH)]
            d = wqe_buf.at[item[1], :, pl.ds(0, NE * DH)]
        return pltpu.make_async_copy(s, d, in_sem.at[sem_idx])

    def out_copy(br, t):
        r0, nr, c = _out_pieces()[t]
        off = br * D + c * QW
        if not isinstance(off, int):
            off = pl.multiple_of(off, QW)
        return pltpu.make_async_copy(out_buf.at[br, pl.ds(r0, nr), pl.ds(c * QW, QW)],
                                     out_hbm.at[pl.ds(r0, nr), pl.ds(off, QW)],
                                     out_sem.at[0])

    def body_views(s):
        return (wql_buf.at[s], k_buf.at[s], v_buf.at[s], wo_buf.at[s, :, pl.ds(0, D)])

    def store_q(step, l, qq):
        qq = (qq * SCALE).astype(jnp.bfloat16)
        if l < NE:
            qe_buf[step * NE + l] = qq
        else:
            ql_buf[step * NL + l - NE] = qq

    @pl.when(i == 0)
    def _startup():
        x_copies = []
        n = 0
        for seg in X_SEGS:
            cps = []
            for item in seg:
                cp = x_copy(item, n)
                cp.start()
                cps.append(cp)
                n += 1
            x_copies.append(cps)
        for s in range(NBODY):
            br, g = divmod(s, NBODY // 2)
            k, v, wo = ((ak, av, awo), (bk, bv, bwo))[br]
            late0 = (s // 2) * G + NE + (s % 2) * NQB
            srcs = (bwq.at[:, pl.ds(late0 * DH, NQB * DH)], k.at[:, pl.ds(g * G, G)],
                    v.at[:, pl.ds(g * G, G)], wo.at[pl.ds(g * G * DH, G * DH), :])
            for j, (src, dst) in enumerate(zip(srcs, body_views(s))):
                pltpu.make_async_copy(src, dst, in_sem.at[NXD + 4 * s + j]).start()

        for si, seg in enumerate(X_SEGS):
            for cp in x_copies[si]:
                cp.wait()
            for item in seg:
                if item[0] == 'w':
                    _, k0, k1, h0, h1 = item
                    for h in range(h0, h1):
                        qq = jnp.dot(x_buf[0, :, k0 * KT:k1 * KT],
                                     wqa_buf[k0 * KT:k1 * KT, h * DH:(h + 1) * DH],
                                     preferred_element_type=jnp.float32)
                        if k0 > 0:
                            qq = qacc[h] + qq
                        if k1 < NK:
                            qacc[h] = qq
                        else:
                            store_q(h // G, h % G, qq)
                elif item[0] == 'wb':
                    for l in range(NE):
                        qq = jnp.dot(x_buf[1], wqe_buf[item[1], :, l * DH:(l + 1) * DH],
                                     preferred_element_type=jnp.float32)
                        store_q(NBODY // 2 + item[1], l, qq)

    br = lax.shift_right_logical(i, 1)
    last = (i & 1) == 1
    for j, view in enumerate(body_views(i)):
        pltpu.make_async_copy(view, view, in_sem.at[NXD + 4 * i + j]).wait()

    row = lax.broadcasted_iota(jnp.int32, (128, 128), 0) // SQ
    col = lax.broadcasted_iota(jnp.int32, (128, 128), 1) // SK
    mask = row == col
    p = {}

    def qproj(j):
        qq = jnp.dot(x_buf[1], wql_buf[i, :, j * DH:(j + 1) * DH],
                     preferred_element_type=jnp.float32)
        ql_buf[2 * NL + NQB * i + j] = (qq * SCALE).astype(jnp.bfloat16)

    def scores(l):
        for j in range(4):
            rows = pl.ds(j * 128, 128)
            if l < NE:
                qs = qe_buf[i * NE + l, rows, :]
            else:
                qs = ql_buf[i * NL + l - NE, rows, :]
            ks = k_buf[i, pl.ds(4 * j, 4), l].reshape(128, DH)
            sc = lax.dot_general(qs, ks, (((1,), (1,)), ((), ())),
                                 preferred_element_type=jnp.float32)
            sc = jnp.where(mask, sc, -jnp.inf)
            m = jnp.max(sc, axis=-1, keepdims=True)
            e = jnp.exp2(sc - m)
            den = jnp.sum(e, axis=-1, keepdims=True)
            p[l, j] = (e.astype(jnp.bfloat16), pl.reciprocal(den, approx=True))

    def pv(l):
        for j in range(4):
            vs = v_buf[i, pl.ds(4 * j, 4), l].reshape(128, DH)
            e, r = p.pop((l, j))
            oo = jnp.dot(e, vs, preferred_element_type=jnp.float32)
            o_buf[l, j * 128:(j + 1) * 128, :] = (oo * r).astype(jnp.bfloat16)

    def oproj(u, c):
        lhs = jnp.concatenate([o_buf[u * U + t] for t in range(U)], axis=1)
        cs = slice(c * QW, (c + 1) * QW)
        y = jnp.dot(lhs, wo_buf[i, u * U * DH:(u + 1) * U * DH, cs],
                    preferred_element_type=jnp.float32)
        prev = acc[:, cs]
        if u == 0:
            prev = jnp.where(last, prev, 0.0)
        y = prev + y
        acc[:, cs] = y
        if u == G // U - 1:
            for t, (r0, nr, pc) in enumerate(_out_pieces()):
                if pc != c:
                    continue
                out_buf[br, r0:r0 + nr, cs] = y[r0:r0 + nr].astype(jnp.bfloat16)

                @pl.when(last)
                def _():
                    out_copy(br, t).start()

    for tok in LOOP_ORDER.split():
        kind, arg = tok[0], tok[1:]
        if kind == 'Q':
            qproj(int(arg))
        elif kind == 'S':
            scores(int(arg))
        elif kind == 'P':
            pv(int(arg))
        else:
            oproj(*(int(v) for v in arg.split('.')))

    @pl.when(i == NBODY - 1)
    def _finish():
        pltpu.make_async_copy(out_hbm, out_hbm, out_sem.at[0]).wait()


@jax.jit
def pallas_concat_heads__mha_block_cached__mha_block_cached__near_ridge_kernel(
    A_x, A_k_cache, A_v_cache, A_wq, A_wo, B_x, B_k_cache, B_v_cache, B_wq, B_wo):
    bf = jnp.bfloat16
    any_spec = pl.BlockSpec(memory_space=pl.ANY)
    out = pl.pallas_call(
        _kernel,
        grid=(NBODY,),
        out_shape=jax.ShapeDtypeStruct((M, 2 * D), bf),
        in_specs=[any_spec] * 10,
        out_specs=any_spec,
        scratch_shapes=[
            pltpu.VMEM((2, M, D), bf),
            pltpu.VMEM((D, H * DH + PAD), bf),
            pltpu.VMEM((2, D, NE * DH + PAD), bf),
            pltpu.VMEM((NBODY, D, NQB * DH), bf),
            pltpu.VMEM((NBODY, B, G, SK, DH), bf),
            pltpu.VMEM((NBODY, B, G, SK, DH), bf),
            pltpu.VMEM((NBODY, G * DH, D + PAD), bf),
            pltpu.VMEM((H, M, DH), jnp.float32),
            pltpu.VMEM((NBODY * NE, M, DH), bf),
            pltpu.VMEM((NBODY * NL, M, DH), bf),
            pltpu.VMEM((G, M, DH), bf),
            pltpu.VMEM((M, D), jnp.float32),
            pltpu.VMEM((2, M, D), bf),
            pltpu.SemaphoreType.DMA((NDMA,)),
            pltpu.SemaphoreType.DMA((1,)),
        ],
        compiler_params=pltpu.CompilerParams(
            dimension_semantics=("arbitrary",),
            vmem_limit_bytes=110 * 1024 * 1024,
            disable_bounds_checks=True,
            disable_semaphore_checks=True),
    )(A_x.reshape(M, D), A_k_cache, A_v_cache, A_wq, A_wo,
      B_x.reshape(M, D), B_k_cache, B_v_cache, B_wq, B_wo)
    return out.reshape(B, SQ, 2 * D)
```

```python
import jax
import jax.numpy as jnp
from jax import lax
import jax.experimental.pallas as pl
import jax.experimental.pallas.tpu as pltpu

B, SQ, D = 16, 32, 1024
H, SK, DH = 32, 32, 128
M = B * SQ
TB = 128 // SQ
G = 16
NSTEP = 2 * H // G
NE = 6
NL = G - NE
NQB = 5
U = 4
NQ = 4
QW = D // NQ
KT = 128
NK = D // KT
NR = 16
PAD = 128
SCALE = (DH ** -0.5) * 1.4426950408889634

X_SEGS = [
    [('x', 0, 1), ('w', 0, 1, 0, 4)],
    [('w', 0, 1, 4, 12)],
    [('w', 0, 1, 12, 32)],
    [('x', 1, 2), ('w', 1, 2, 0, 32)],
    [('x', 2, 4), ('w', 2, 4, 0, 28)],
    [('w', 2, 4, 28, 32), ('x', 4, 7), ('w', 4, 7, 0, 28)],
    [('w', 4, 7, 28, 32), ('x', 7, 8), ('w', 7, 8, 0, 32), ('xb',), ('wb', 0), ('wb', 1)],
]
STEP_ORDER = (
    "Q0 S0 S1 Q1 P0 P1 S2 S3 Q2 P2 P3 S4 S5 Q3 P4 P5 Q4 O0.0 "
    "S6 O0.1 P6 S7 O0.2 P7 S8 O0.3 P8 S9 O1.0 P9 S10 O1.1 P10 S11 O1.2 P11 S12 O1.3 P12 "
    "S13 O2.0 P13 S14 O2.1 P14 S15 O2.2 P15 O2.3 O3.0 O3.1 O3.2 O3.3")
NXD = sum(len(seg) for seg in X_SEGS)
NDMA = NXD + 4 * NSTEP
OUT_PIECES = ([(0, M, c) for c in range(NQ - 1)]
              + [(r * (M // NR), M // NR, NQ - 1) for r in range(NR)])


def _kernel(ax, ak, av, awq, awo, bx, bk, bv, bwq, bwo, out_hbm,
            x_buf, wqa_buf, wqe_buf, wql_buf, k_buf, v_buf, wo_buf,
            qacc, qe_buf, ql_buf, o_buf, acc, out_buf, in_sem, out_sem):
    i = pl.program_id(0)
    f32, bf16 = jnp.float32, jnp.bfloat16

    def startup_copy(item, sem_idx):
        kind = item[0]
        if kind == 'x':
            cols = pl.ds(item[1] * KT, (item[2] - item[1]) * KT)
            src, dst = ax.at[:, cols], x_buf.at[0, :, cols]
        elif kind == 'w':
            rows = pl.ds(item[1] * KT, (item[2] - item[1]) * KT)
            cols = pl.ds(item[3] * DH, (item[4] - item[3]) * DH)
            src, dst = awq.at[rows, cols], wqa_buf.at[rows, cols]
        elif kind == 'xb':
            src, dst = bx, x_buf.at[1]
        else:
            src = bwq.at[:, pl.ds(item[1] * G * DH, NE * DH)]
            dst = wqe_buf.at[item[1], :, pl.ds(0, NE * DH)]
        return pltpu.make_async_copy(src, dst, in_sem.at[sem_idx])

    def step_views(s):
        return (wql_buf.at[s], k_buf.at[s], v_buf.at[s], wo_buf.at[s, :, pl.ds(0, D)])

    def store_q(s, l, q):
        if l < NE:
            qe_buf[s * NE + l] = q.astype(bf16)
        else:
            ql_buf[s * NL + l - NE] = q.astype(bf16)

    @pl.when(i == 0)
    def _startup():
        seg_copies = []
        n = 0
        for seg in X_SEGS:
            seg_copies.append([startup_copy(item, n + t) for t, item in enumerate(seg)])
            n += len(seg)
            for cp in seg_copies[-1]:
                cp.start()
        for s in range(NSTEP):
            br, g = divmod(s, NSTEP // 2)
            k, v, wo = ((ak, av, awo), (bk, bv, bwo))[br]
            late0 = (s // 2) * G + NE + (s % 2) * NQB
            srcs = (bwq.at[:, pl.ds(late0 * DH, NQB * DH)], k.at[:, pl.ds(g * G, G)],
                    v.at[:, pl.ds(g * G, G)], wo.at[pl.ds(g * G * DH, G * DH), :])
            for j, (src, dst) in enumerate(zip(srcs, step_views(s))):
                pltpu.make_async_copy(src, dst, in_sem.at[NXD + 4 * s + j]).start()

        for seg, copies in zip(X_SEGS, seg_copies):
            for cp in copies:
                cp.wait()
            for item in seg:
                if item[0] == 'w':
                    _, k0, k1, h0, h1 = item
                    for h in range(h0, h1):
                        q = jnp.dot(x_buf[0, :, k0 * KT:k1 * KT],
                                    wqa_buf[k0 * KT:k1 * KT, h * DH:(h + 1) * DH],
                                    preferred_element_type=f32)
                        if k0 > 0:
                            q = qacc[h] + q
                        if k1 < NK:
                            qacc[h] = q
                        else:
                            store_q(h // G, h % G, q)
                elif item[0] == 'wb':
                    for l in range(NE):
                        q = jnp.dot(x_buf[1], wqe_buf[item[1], :, l * DH:(l + 1) * DH],
                                    preferred_element_type=f32)
                        store_q(NSTEP // 2 + item[1], l, q)

    br = lax.shift_right_logical(i, 1)
    last = (i & 1) == 1
    for j, view in enumerate(step_views(i)):
        pltpu.make_async_copy(view, view, in_sem.at[NXD + 4 * i + j]).wait()

    row = lax.broadcasted_iota(jnp.int32, (TB * SQ, TB * SK), 0) // SQ
    col = lax.broadcasted_iota(jnp.int32, (TB * SQ, TB * SK), 1) // SK
    same_batch = row == col
    probs = {}

    def qproj(j):
        q = jnp.dot(x_buf[1], wql_buf[i, :, j * DH:(j + 1) * DH], preferred_element_type=f32)
        ql_buf[(NSTEP // 2) * NL + NQB * i + j] = q.astype(bf16)

    def scores(l):
        for j in range(B // TB):
            rows = pl.ds(j * TB * SQ, TB * SQ)
            if l < NE:
                q = qe_buf[i * NE + l, rows, :]
            else:
                q = ql_buf[i * NL + l - NE, rows, :]
            k = k_buf[i, pl.ds(j * TB, TB), l].reshape(TB * SK, DH)
            s = lax.dot_general(q, k, (((1,), (1,)), ((), ())), preferred_element_type=f32)
            s = jnp.where(same_batch, s, -jnp.inf)
            e = jnp.exp2((s - jnp.max(s, axis=-1, keepdims=True)) * SCALE)
            den = jnp.sum(e, axis=-1, keepdims=True)
            probs[l, j] = (e.astype(bf16), pl.reciprocal(den, approx=True))

    def pv(l):
        for j in range(B // TB):
            v = v_buf[i, pl.ds(j * TB, TB), l].reshape(TB * SK, DH)
            e, inv = probs.pop((l, j))
            o = jnp.dot(e, v, preferred_element_type=f32) * inv
            o_buf[l, j * TB * SQ:(j + 1) * TB * SQ, :] = o.astype(bf16)

    def oproj(u, c):
        lhs = jnp.concatenate([o_buf[u * U + t] for t in range(U)], axis=1)
        cs = slice(c * QW, (c + 1) * QW)
        y = jnp.dot(lhs, wo_buf[i, u * U * DH:(u + 1) * U * DH, cs], preferred_element_type=f32)
        prev = acc[:, cs]
        if u == 0:
            prev = jnp.where(last, prev, 0.0)
        y = prev + y
        acc[:, cs] = y
        if u < G // U - 1:
            return
        for r0, nr, pc in OUT_PIECES:
            if pc != c:
                continue
            out_buf[br, r0:r0 + nr, cs] = y[r0:r0 + nr].astype(bf16)

            @pl.when(last)
            def _():
                off = pl.multiple_of(br * D + c * QW, QW)
                pltpu.make_async_copy(out_buf.at[br, pl.ds(r0, nr), pl.ds(c * QW, QW)],
                                      out_hbm.at[pl.ds(r0, nr), pl.ds(off, QW)],
                                      out_sem.at[0]).start()

    for tok in STEP_ORDER.split():
        kind, arg = tok[0], tok[1:]
        if kind == 'O':
            oproj(*(int(v) for v in arg.split('.')))
        else:
            {'Q': qproj, 'S': scores, 'P': pv}[kind](int(arg))

    @pl.when(i == NSTEP - 1)
    def _finish():
        pltpu.make_async_copy(out_hbm, out_hbm, out_sem.at[0]).wait()


@jax.jit
def pallas_concat_heads__mha_block_cached__mha_block_cached__near_ridge_kernel(
    A_x: jax.Array,
    A_k_cache: jax.Array,
    A_v_cache: jax.Array,
    A_wq: jax.Array,
    A_wo: jax.Array,
    B_x: jax.Array,
    B_k_cache: jax.Array,
    B_v_cache: jax.Array,
    B_wq: jax.Array,
    B_wo: jax.Array,
):
    bf16 = jnp.bfloat16
    hbm = pl.BlockSpec(memory_space=pl.ANY)
    out = pl.pallas_call(
        _kernel,
        grid=(NSTEP,),
        out_shape=jax.ShapeDtypeStruct((M, 2 * D), bf16),
        in_specs=[hbm] * 10,
        out_specs=hbm,
        scratch_shapes=[
            pltpu.VMEM((2, M, D), bf16),
            pltpu.VMEM((D, H * DH + PAD), bf16),
            pltpu.VMEM((2, D, NE * DH + PAD), bf16),
            pltpu.VMEM((NSTEP, D, NQB * DH), bf16),
            pltpu.VMEM((NSTEP, B, G, SK, DH), bf16),
            pltpu.VMEM((NSTEP, B, G, SK, DH), bf16),
            pltpu.VMEM((NSTEP, G * DH, D + PAD), bf16),
            pltpu.VMEM((H, M, DH), jnp.float32),
            pltpu.VMEM((NSTEP * NE, M, DH), bf16),
            pltpu.VMEM((NSTEP * NL, M, DH), bf16),
            pltpu.VMEM((G, M, DH), bf16),
            pltpu.VMEM((M, D), jnp.float32),
            pltpu.VMEM((2, M, D), bf16),
            pltpu.SemaphoreType.DMA((NDMA,)),
            pltpu.SemaphoreType.DMA((1,)),
        ],
        compiler_params=pltpu.CompilerParams(
            dimension_semantics=("arbitrary",),
            vmem_limit_bytes=110 * 1024 * 1024,
            disable_bounds_checks=True,
            disable_semaphore_checks=True),
    )(A_x.reshape(M, D), A_k_cache, A_v_cache, A_wq, A_wo,
      B_x.reshape(M, D), B_k_cache, B_v_cache, B_wq, B_wo)
    return out.reshape(B, SQ, 2 * D)
```

```python
import jax
import jax.numpy as jnp
from jax import lax
import jax.experimental.pallas as pl
import jax.experimental.pallas.tpu as pltpu

B, SQ, D = 16, 32, 1024
H, SK, DH = 32, 32, 128
M = B * SQ
TB = 128 // SQ
G = 16
NSTEP = 2 * H // G
NE = 6
NL = G - NE
NQB = 5
U = 4
NQ = 4
QW = D // NQ
FW = 128
KT = 128
NK = D // KT
NR = 16
PAD = 128
SCALE = (DH ** -0.5) * 1.4426950408889634

X_SEGS = [
    [('x', 0, 1), ('w', 0, 1, 0, 4)],
    [('w', 0, 1, 4, 12)],
    [('w', 0, 1, 12, 32)],
    [('x', 1, 2), ('w', 1, 2, 0, 32)],
    [('x', 2, 4), ('w', 2, 4, 0, 28)],
    [('w', 2, 4, 28, 32), ('x', 4, 7), ('w', 4, 7, 0, 28)],
    [('w', 4, 7, 28, 32), ('x', 7, 8), ('w', 7, 8, 0, 32), ('xb',), ('wb', 0), ('wb', 1)],
]
STEP_ORDER = (
    "Q0 S0 S1 Q1 P0 P1 S2 S3 Q2 P2 P3 S4 S5 Q3 P4 P5 Q4 O0.0 "
    "S6 O0.1 P6 S7 O0.2 P7 S8 O0.3 P8 S9 O1.0 P9 S10 O1.1 P10 S11 O1.2 P11 S12 O1.3 P12 "
    "S13 O2.0 P13 S14 O2.1 P14 S15 O2.2 P15 O2.3 F0 F1 F2 F3 F4 F5 F6 F7")
NXD = sum(len(seg) for seg in X_SEGS)
NDMA = NXD + 4 * NSTEP


def _kernel(ax, ak, av, awq, awo, bx, bk, bv, bwq, bwo, out_hbm,
            x_buf, wqa_buf, wqe_buf, wql_buf, k_buf, v_buf, wo_buf,
            qacc, qe_buf, ql_buf, o_buf, acc, out_buf, in_sem, out_sem):
    i = pl.program_id(0)
    f32, bf16 = jnp.float32, jnp.bfloat16

    def startup_copy(item, sem_idx):
        kind = item[0]
        if kind == 'x':
            cols = pl.ds(item[1] * KT, (item[2] - item[1]) * KT)
            src, dst = ax.at[:, cols], x_buf.at[0, :, cols]
        elif kind == 'w':
            rows = pl.ds(item[1] * KT, (item[2] - item[1]) * KT)
            cols = pl.ds(item[3] * DH, (item[4] - item[3]) * DH)
            src, dst = awq.at[rows, cols], wqa_buf.at[rows, cols]
        elif kind == 'xb':
            src, dst = bx, x_buf.at[1]
        else:
            src = bwq.at[:, pl.ds(item[1] * G * DH, NE * DH)]
            dst = wqe_buf.at[item[1], :, pl.ds(0, NE * DH)]
        return pltpu.make_async_copy(src, dst, in_sem.at[sem_idx])

    def step_views(s):
        return (wql_buf.at[s], k_buf.at[s], v_buf.at[s], wo_buf.at[s, :, pl.ds(0, D)])

    def store_q(s, l, q):
        if l < NE:
            qe_buf[s * NE + l] = q.astype(bf16)
        else:
            ql_buf[s * NL + l - NE] = q.astype(bf16)

    @pl.when(i == 0)
    def _startup():
        seg_copies = []
        n = 0
        for seg in X_SEGS:
            seg_copies.append([startup_copy(item, n + t) for t, item in enumerate(seg)])
            n += len(seg)
            for cp in seg_copies[-1]:
                cp.start()
        for s in range(NSTEP):
            br, g = divmod(s, NSTEP // 2)
            k, v, wo = ((ak, av, awo), (bk, bv, bwo))[br]
            late0 = (s // 2) * G + NE + (s % 2) * NQB
            srcs = (bwq.at[:, pl.ds(late0 * DH, NQB * DH)], k.at[:, pl.ds(g * G, G)],
                    v.at[:, pl.ds(g * G, G)], wo.at[pl.ds(g * G * DH, G * DH), :])
            for j, (src, dst) in enumerate(zip(srcs, step_views(s))):
                pltpu.make_async_copy(src, dst, in_sem.at[NXD + 4 * s + j]).start()

        for seg, copies in zip(X_SEGS, seg_copies):
            for cp in copies:
                cp.wait()
            for item in seg:
                if item[0] == 'w':
                    _, k0, k1, h0, h1 = item
                    xk = x_buf[0, :, k0 * KT:k1 * KT]
                    for h in range(h0, h1):
                        q = jnp.dot(xk, wqa_buf[k0 * KT:k1 * KT, h * DH:(h + 1) * DH],
                                    preferred_element_type=f32)
                        if k0 > 0:
                            q = qacc[h] + q
                        if k1 < NK:
                            qacc[h] = q
                        else:
                            store_q(h // G, h % G, q)
                elif item[0] == 'xb':
                    xb = x_buf[1]
                elif item[0] == 'wb':
                    for l in range(NE):
                        q = jnp.dot(xb, wqe_buf[item[1], :, l * DH:(l + 1) * DH],
                                    preferred_element_type=f32)
                        store_q(NSTEP // 2 + item[1], l, q)

    br = lax.shift_right_logical(i, 1)
    last = (i & 1) == 1
    for j, view in enumerate(step_views(i)):
        pltpu.make_async_copy(view, view, in_sem.at[NXD + 4 * i + j]).wait()

    row = lax.broadcasted_iota(jnp.int32, (TB * SQ, TB * SK), 0) // SQ
    col = lax.broadcasted_iota(jnp.int32, (TB * SQ, TB * SK), 1) // SK
    same_batch = row == col
    probs = {}
    xb = x_buf[1]
    units = {}

    def qproj(j):
        q = jnp.dot(xb, wql_buf[i, :, j * DH:(j + 1) * DH], preferred_element_type=f32)
        ql_buf[(NSTEP // 2) * NL + NQB * i + j] = q.astype(bf16)

    def scores(l):
        for j in range(B // TB):
            rows = pl.ds(j * TB * SQ, TB * SQ)
            if l < NE:
                q = qe_buf[i * NE + l, rows, :]
            else:
                q = ql_buf[i * NL + l - NE, rows, :]
            k = k_buf[i, pl.ds(j * TB, TB), l].reshape(TB * SK, DH)
            s = lax.dot_general(q, k, (((1,), (1,)), ((), ())), preferred_element_type=f32)
            s = jnp.where(same_batch, s, -jnp.inf)
            e = jnp.exp2((s - jnp.max(s, axis=-1, keepdims=True)) * SCALE)
            den = jnp.sum(e, axis=-1, keepdims=True)
            probs[l, j] = (e.astype(bf16), pl.reciprocal(den, approx=True))

    def pv(l):
        for j in range(B // TB):
            v = v_buf[i, pl.ds(j * TB, TB), l].reshape(TB * SK, DH)
            e, inv = probs.pop((l, j))
            o = jnp.dot(e, v, preferred_element_type=f32) * inv
            o_buf[l, j * TB * SQ:(j + 1) * TB * SQ, :] = o.astype(bf16)

    def oproj(u, c, width=QW):
        if u not in units:
            units[u] = jnp.concatenate([o_buf[u * U + t] for t in range(U)], axis=1)
        lhs = units[u]
        cs = slice(c * width, (c + 1) * width)
        y = jnp.dot(lhs, wo_buf[i, u * U * DH:(u + 1) * U * DH, cs], preferred_element_type=f32)
        prev = acc[:, cs]
        if u == 0:
            prev = jnp.where(last, prev, 0.0)
        y = prev + y
        acc[:, cs] = y
        return y

    def oproj_final(c):
        y = oproj(G // U - 1, c, FW).astype(bf16)
        nr = M // NR if c == D // FW - 1 else M
        for r0 in range(0, M, nr):
            out_buf[br, r0:r0 + nr, c * FW:(c + 1) * FW] = y[r0:r0 + nr]

            @pl.when(last)
            def _():
                off = pl.multiple_of(br * D + c * FW, FW)
                pltpu.make_async_copy(out_buf.at[br, pl.ds(r0, nr), pl.ds(c * FW, FW)],
                                      out_hbm.at[pl.ds(r0, nr), pl.ds(off, FW)],
                                      out_sem.at[0]).start()

    for tok in STEP_ORDER.split():
        kind, arg = tok[0], tok[1:]
        if kind == 'O':
            oproj(*(int(v) for v in arg.split('.')))
        else:
            {'Q': qproj, 'S': scores, 'P': pv, 'F': oproj_final}[kind](int(arg))

    @pl.when(i == NSTEP - 1)
    def _finish():
        pltpu.make_async_copy(out_hbm, out_hbm, out_sem.at[0]).wait()


@jax.jit
def pallas_concat_heads__mha_block_cached__mha_block_cached__near_ridge_kernel(
    A_x: jax.Array,
    A_k_cache: jax.Array,
    A_v_cache: jax.Array,
    A_wq: jax.Array,
    A_wo: jax.Array,
    B_x: jax.Array,
    B_k_cache: jax.Array,
    B_v_cache: jax.Array,
    B_wq: jax.Array,
    B_wo: jax.Array,
):
    bf16 = jnp.bfloat16
    hbm = pl.BlockSpec(memory_space=pl.ANY)
    out = pl.pallas_call(
        _kernel,
        grid=(NSTEP,),
        out_shape=jax.ShapeDtypeStruct((M, 2 * D), bf16),
        in_specs=[hbm] * 10,
        out_specs=hbm,
        scratch_shapes=[
            pltpu.VMEM((2, M, D), bf16),
            pltpu.VMEM((D, H * DH + PAD), bf16),
            pltpu.VMEM((2, D, NE * DH + PAD), bf16),
            pltpu.VMEM((NSTEP, D, NQB * DH), bf16),
            pltpu.VMEM((NSTEP, B, G, SK, DH), bf16),
            pltpu.VMEM((NSTEP, B, G, SK, DH), bf16),
            pltpu.VMEM((NSTEP, G * DH, D + PAD), bf16),
            pltpu.VMEM((H, M, DH), jnp.float32),
            pltpu.VMEM((NSTEP * NE, M, DH), bf16),
            pltpu.VMEM((NSTEP * NL, M, DH), bf16),
            pltpu.VMEM((G, M, DH), bf16),
            pltpu.VMEM((M, D), jnp.float32),
            pltpu.VMEM((2, M, D), bf16),
            pltpu.SemaphoreType.DMA((NDMA,)),
            pltpu.SemaphoreType.DMA((1,)),
        ],
        compiler_params=pltpu.CompilerParams(
            dimension_semantics=("arbitrary",),
            vmem_limit_bytes=110 * 1024 * 1024,
            disable_bounds_checks=True,
            disable_semaphore_checks=True),
    )(A_x.reshape(M, D), A_k_cache, A_v_cache, A_wq, A_wo,
      B_x.reshape(M, D), B_k_cache, B_v_cache, B_wq, B_wo)
    return out.reshape(B, SQ, 2 * D)
```

```python
import jax
import jax.numpy as jnp
from jax import lax
import jax.experimental.pallas as pl
import jax.experimental.pallas.tpu as pltpu

B, SQ, D = 16, 32, 1024
H, SK, DH = 32, 32, 128
M = B * SQ
TB = 128 // SQ
G = 16
NSTEP = 2 * H // G
NE = 6
NL = G - NE
NQB = 5
U = 4
NQ = 4
QW = D // NQ
FW = 128
KT = 128
NK = D // KT
NR = 16
PAD = 128
SCALE = (DH ** -0.5) * 1.4426950408889634

X_SEGS = [
    [('x', 0, 1), ('w', 0, 1, 0, 4)],
    [('w', 0, 1, 4, 12)],
    [('w', 0, 1, 12, 32)],
    [('x', 1, 2), ('w', 1, 2, 0, 32)],
    [('x', 2, 4), ('w', 2, 4, 0, 28)],
    [('w', 2, 4, 28, 32), ('x', 4, 7), ('w', 4, 7, 0, 28)],
    [('w', 4, 7, 28, 32), ('x', 7, 8), ('w', 7, 8, 0, 32), ('xb',), ('wb', 0), ('wb', 1)],
]
STEP_ORDER = (
    "Q0 S0 S1 Q1 P0 P1 S2 S3 Q2 P2 P3 S4 S5 Q3 P4 P5 Q4 O0.0 "
    "S6 O0.1 P6 S7 O0.2 P7 S8 O0.3 P8 S9 O1.0 P9 S10 O1.1 P10 S11 O1.2 P11 S12 O1.3 P12 "
    "S13 O2.0 P13 S14 O2.1 P14 S15 O2.2 P15 O2.3 F0 F1 F2 F3 F4 F5 F6 F7")
NXD = sum(len(seg) for seg in X_SEGS)
NDMA = NXD + 4 * NSTEP


def _kernel(ax, ak, av, awq, awo, bx, bk, bv, bwq, bwo, out_hbm,
            x_buf, wqa_buf, wqe_buf, wql_buf, k_buf, v_buf, wo_buf,
            qacc, qe_buf, ql_buf, o_buf, acc, out_buf, in_sem, out_sem):
    i = pl.program_id(0)
    f32, bf16 = jnp.float32, jnp.bfloat16

    def startup_copy(item, sem_idx):
        kind = item[0]
        if kind == 'x':
            cols = pl.ds(item[1] * KT, (item[2] - item[1]) * KT)
            src, dst = ax.at[:, cols], x_buf.at[0, :, cols]
        elif kind == 'w':
            rows = pl.ds(item[1] * KT, (item[2] - item[1]) * KT)
            cols = pl.ds(item[3] * DH, (item[4] - item[3]) * DH)
            src, dst = awq.at[rows, cols], wqa_buf.at[rows, cols]
        elif kind == 'xb':
            src, dst = bx, x_buf.at[1]
        else:
            src = bwq.at[:, pl.ds(item[1] * G * DH, NE * DH)]
            dst = wqe_buf.at[item[1], :, pl.ds(0, NE * DH)]
        return pltpu.make_async_copy(src, dst, in_sem.at[sem_idx])

    def step_views(s):
        return (wql_buf.at[s], k_buf.at[s], v_buf.at[s], wo_buf.at[s, :, pl.ds(0, D)])

    def store_q(s, l, q):
        if l < NE:
            qe_buf[s * NE + l] = q.astype(bf16)
        else:
            ql_buf[s * NL + l - NE] = q.astype(bf16)

    @pl.when(i == 0)
    def _startup():
        seg_copies = []
        n = 0
        for seg in X_SEGS:
            seg_copies.append([startup_copy(item, n + t) for t, item in enumerate(seg)])
            n += len(seg)
            for cp in seg_copies[-1]:
                cp.start()
        for s in range(NSTEP):
            br, g = divmod(s, NSTEP // 2)
            k, v, wo = ((ak, av, awo), (bk, bv, bwo))[br]
            late0 = (s // 2) * G + NE + (s % 2) * NQB
            srcs = (bwq.at[:, pl.ds(late0 * DH, NQB * DH)], k.at[:, pl.ds(g * G, G)],
                    v.at[:, pl.ds(g * G, G)], wo.at[pl.ds(g * G * DH, G * DH), :])
            for j, (src, dst) in enumerate(zip(srcs, step_views(s))):
                pltpu.make_async_copy(src, dst, in_sem.at[NXD + 4 * s + j]).start()

        acc[...] = jnp.zeros(acc.shape, f32)

        for seg, copies in zip(X_SEGS, seg_copies):
            for cp in copies:
                cp.wait()
            for item in seg:
                if item[0] == 'w':
                    _, k0, k1, h0, h1 = item
                    xk = x_buf[0, :, k0 * KT:k1 * KT]
                    for h in range(h0, h1):
                        q = jnp.dot(xk, wqa_buf[k0 * KT:k1 * KT, h * DH:(h + 1) * DH],
                                    preferred_element_type=f32)
                        if k0 > 0:
                            q = qacc[h] + q
                        if k1 < NK:
                            qacc[h] = q
                        else:
                            store_q(h // G, h % G, q)
                elif item[0] == 'xb':
                    xb = x_buf[1]
                elif item[0] == 'wb':
                    for l in range(NE):
                        q = jnp.dot(xb, wqe_buf[item[1], :, l * DH:(l + 1) * DH],
                                    preferred_element_type=f32)
                        store_q(NSTEP // 2 + item[1], l, q)

    br = lax.shift_right_logical(i, 1)
    last = (i & 1) == 1
    for j, view in enumerate(step_views(i)):
        pltpu.make_async_copy(view, view, in_sem.at[NXD + 4 * i + j]).wait()

    row = lax.broadcasted_iota(jnp.int32, (TB * SQ, TB * SK), 0) // SQ
    col = lax.broadcasted_iota(jnp.int32, (TB * SQ, TB * SK), 1) // SK
    same_batch = row == col
    probs = {}
    xb = x_buf[1]
    units = {}

    def qproj(j):
        q = jnp.dot(xb, wql_buf[i, :, j * DH:(j + 1) * DH], preferred_element_type=f32)
        ql_buf[(NSTEP // 2) * NL + NQB * i + j] = q.astype(bf16)

    def scores(l):
        for j in range(B // TB):
            rows = pl.ds(j * TB * SQ, TB * SQ)
            if l < NE:
                q = qe_buf[i * NE + l, rows, :]
            else:
                q = ql_buf[i * NL + l - NE, rows, :]
            k = k_buf[i, pl.ds(j * TB, TB), l].reshape(TB * SK, DH)
            s = lax.dot_general(q, k, (((1,), (1,)), ((), ())), preferred_element_type=f32)
            s = jnp.where(same_batch, s, -jnp.inf)
            e = jnp.exp2((s - jnp.max(s, axis=-1, keepdims=True)) * SCALE)
            den = jnp.sum(e, axis=-1, keepdims=True)
            inv = pl.reciprocal(den, approx=True)
            inv = inv * (2.0 - den * inv)
            probs[l, j] = (e.astype(bf16), inv)

    def pv(l):
        for j in range(B // TB):
            v = v_buf[i, pl.ds(j * TB, TB), l].reshape(TB * SK, DH)
            e, inv = probs.pop((l, j))
            o = jnp.dot(e, v, preferred_element_type=f32) * inv
            o_buf[l, j * TB * SQ:(j + 1) * TB * SQ, :] = o.astype(bf16)

    def oproj(u, c, width=QW):
        if u not in units:
            units[u] = jnp.concatenate([o_buf[u * U + t] for t in range(U)], axis=1)
        lhs = units[u]
        cs = slice(c * width, (c + 1) * width)
        y = jnp.dot(lhs, wo_buf[i, u * U * DH:(u + 1) * U * DH, cs], preferred_element_type=f32)
        prev = acc[:, cs]
        if u == 0:
            prev = jnp.where(last, prev, 0.0)
        y = prev + y
        acc[:, cs] = y
        return y

    def oproj_final(c):
        y = oproj(G // U - 1, c, FW).astype(bf16)
        nr = M // NR if c == D // FW - 1 else M
        for r0 in range(0, M, nr):
            out_buf[br, r0:r0 + nr, c * FW:(c + 1) * FW] = y[r0:r0 + nr]

            @pl.when(last)
            def _():
                off = pl.multiple_of(br * D + c * FW, FW)
                pltpu.make_async_copy(out_buf.at[br, pl.ds(r0, nr), pl.ds(c * FW, FW)],
                                      out_hbm.at[pl.ds(r0, nr), pl.ds(off, FW)],
                                      out_sem.at[0]).start()

    for tok in STEP_ORDER.split():
        kind, arg = tok[0], tok[1:]
        if kind == 'O':
            oproj(*(int(v) for v in arg.split('.')))
        else:
            {'Q': qproj, 'S': scores, 'P': pv, 'F': oproj_final}[kind](int(arg))

    @pl.when(i == NSTEP - 1)
    def _finish():
        pltpu.make_async_copy(out_hbm, out_hbm, out_sem.at[0]).wait()


@jax.jit
def pallas_concat_heads__mha_block_cached__mha_block_cached__near_ridge_kernel(
    A_x: jax.Array,
    A_k_cache: jax.Array,
    A_v_cache: jax.Array,
    A_wq: jax.Array,
    A_wo: jax.Array,
    B_x: jax.Array,
    B_k_cache: jax.Array,
    B_v_cache: jax.Array,
    B_wq: jax.Array,
    B_wo: jax.Array,
):
    bf16 = jnp.bfloat16
    hbm = pl.BlockSpec(memory_space=pl.ANY)
    out = pl.pallas_call(
        _kernel,
        grid=(NSTEP,),
        out_shape=jax.ShapeDtypeStruct((M, 2 * D), bf16),
        in_specs=[hbm] * 10,
        out_specs=hbm,
        scratch_shapes=[
            pltpu.VMEM((2, M, D), bf16),
            pltpu.VMEM((D, H * DH + PAD), bf16),
            pltpu.VMEM((2, D, NE * DH + PAD), bf16),
            pltpu.VMEM((NSTEP, D, NQB * DH), bf16),
            pltpu.VMEM((NSTEP, B, G, SK, DH), bf16),
            pltpu.VMEM((NSTEP, B, G, SK, DH), bf16),
            pltpu.VMEM((NSTEP, G * DH, D + PAD), bf16),
            pltpu.VMEM((H, M, DH), jnp.float32),
            pltpu.VMEM((NSTEP * NE, M, DH), bf16),
            pltpu.VMEM((NSTEP * NL, M, DH), bf16),
            pltpu.VMEM((G, M, DH), bf16),
            pltpu.VMEM((M, D), jnp.float32),
            pltpu.VMEM((2, M, D), bf16),
            pltpu.SemaphoreType.DMA((NDMA,)),
            pltpu.SemaphoreType.DMA((1,)),
        ],
        compiler_params=pltpu.CompilerParams(
            dimension_semantics=("arbitrary",),
            vmem_limit_bytes=110 * 1024 * 1024,
            disable_bounds_checks=True,
            disable_semaphore_checks=True),
    )(A_x.reshape(M, D), A_k_cache, A_v_cache, A_wq, A_wo,
      B_x.reshape(M, D), B_k_cache, B_v_cache, B_wq, B_wo)
    return out.reshape(B, SQ, 2 * D)
```
